```python
import jax
import jax.numpy as jnp

def _softmax(x, axis=-1):
    return jax.nn.softmax(x, axis=axis)
def _gelu(x):
    return jax.nn.gelu(x, approximate=True)
def _silu(x):
    return jax.nn.silu(x)
def _sigmoid(x):
    return jax.nn.sigmoid(x)
def _layernorm(x, axis=-1, eps=1e-5):
    m = jnp.mean(x, axis=axis, keepdims=True)
    v = jnp.var(x, axis=axis, keepdims=True)
    return (x - m) / jnp.sqrt(v + eps)
def _scatter_add(tgt, idx, src, axis=0):
    return tgt.at[idx].add(src)
def _segment_sum(src, seg, n):
    return jax.ops.segment_sum(src, seg, n)
class _Rng:
    def __init__(self, key):
        self._k = key
    def _next(self):
        self._k, sub = jax.random.split(self._k)
        return sub
    def normal(self, shape):
        return jax.random.normal(self._next(), shape, dtype=jnp.bfloat16)
    def randint(self, lo, hi, shape):
        return jax.random.randint(self._next(), shape, lo, hi, dtype=jnp.int32)
    def uniform(self, shape, lo=0.0, hi=1.0):
        return jax.random.uniform(self._next(), shape, jnp.bfloat16, lo, hi)
    def permutation(self, n):
        return jax.random.permutation(self._next(), n)


kernel_name = 'interleave_layers__sliding_local_dilated__spectral_gfnet__prompt'

def setup_inputs():
    _rng = _Rng(jax.random.key(int.from_bytes(__import__("os").urandom(4), "little")))
    _w = (lambda a: (lambda t: t.astype(jnp.bfloat16) if jnp.issubdtype(t.dtype, jnp.floating) else t)(jnp.asarray(a)))
    def _A_setup():
        B, S, D = 1, 2048, 1024
        return {
            "x": _w((lambda *s: _rng.normal(s) * 0.05)(B, S, D)),
            "wqkv": _w((lambda *s: _rng.normal(s) * 0.05)(D, 3 * D)),
            "wo": _w((lambda *s: _rng.normal(s) * 0.05)(D, D)),
        }
    _A_in = _A_setup()

    def _B_setup():
        B, S, D = 1, 2048, 1024
        Df = D // 2 + 1
        return {
            "x": _w((lambda *s: _rng.normal(s) * 0.05)(B, S, D)),
            "w_r": _w((lambda *s: _rng.normal(s) * 0.05)(S, Df) * 0.02),
            "w_i": _w((lambda *s: _rng.normal(s) * 0.05)(S, Df) * 0.02),
        }
    _B_in = _B_setup()

    return {
        "A_x": _A_in["x"],
        "A_wqkv": _A_in["wqkv"],
        "A_wo": _A_in["wo"],
        "B_x": _B_in["x"],
        "B_w_r": _B_in["w_r"],
        "B_w_i": _B_in["w_i"],
    }

def reference(A_x, A_wqkv, A_wo, B_x, B_w_r, B_w_i):
    def _A_ref(x, wqkv, wo):
        B, S, D = x.shape
        H = 32; Dh = D // H
        W, dil = 8, 2
        qkv = (lambda x, *d: x.transpose(*d))((x @ wqkv).reshape(B, S, 3, H, Dh), 2, 0, 3, 1, 4)
        q, k, v = qkv[0], qkv[1], qkv[2]
        scale = Dh ** -0.5
        pos = jnp.arange(S)
        off = jnp.arange(W) * dil
        idx = pos[:, None] - off[None, :]
        mask = idx >= 0
        idx_c = jnp.where(mask, idx, 0).reshape(-1)
        kg = k[:, :, idx_c, :].reshape(B, H, S, W, Dh)
        vg = v[:, :, idx_c, :].reshape(B, H, S, W, Dh)
        logits = jnp.einsum("bhsd,bhswd->bhsw", q, kg) * scale
        logits = jnp.where(mask[None, None, :, :], logits, -1e9)
        attn = _softmax(logits, axis=-1)
        o = jnp.einsum("bhsw,bhswd->bhsd", attn, vg)
        return (lambda x, *d: x.transpose(*d))(o, 0, 2, 1, 3).reshape(B, S, D) @ wo

    def _B_ref(x, w_r, w_i):
        B, S, D = x.shape
        X = (lambda x, axes=(-2,-1): jnp.fft.rfft2(x.astype(jnp.float32), axes=axes))(x, axes=(-2, -1))
        W = w_r + 1j * w_i
        X = X * W
        y = (lambda x, s, axes=(-2,-1): jnp.fft.irfft2(x, s=s, axes=axes).astype(jnp.bfloat16))(X, (S, D), axes=(-2, -1))
        return y

    x = A_x
    x = x + _A_ref(_layernorm(x, axis=-1), A_wqkv, A_wo)
    x = x + _B_ref(_layernorm(x, axis=-1), B_w_r, B_w_i)
    x = x + _A_ref(_layernorm(x, axis=-1), A_wqkv, A_wo)
    x = x + _B_ref(_layernorm(x, axis=-1), B_w_r, B_w_i)
    return x
```

```python
import numpy as np
import jax
import jax.numpy as jnp
from jax import lax
import jax.experimental.pallas as pl
import jax.experimental.pallas.tpu as pltpu

S, D, H, DH, NW = 2048, 1024, 32, 32, 8
T, L = 16, 128
RES = (0, 4, 1, 7, 2, 6, 3, 5)
ZR = 528
F32, BF16 = jnp.float32, jnp.bfloat16


def _cplx_rhs(m):
    return np.block([[m.real, m.imag], [-m.imag, m.real]])


def _consts():
    l = np.arange(L)[:, None]
    k = np.arange(L)[None, :]
    fs = [np.exp(-2j * np.pi * (((T * l + t) * k) % S) / S) for t in range(T)]
    sf = np.stack([_cplx_rhs(f) for f in fs])
    si = np.stack([_cplx_rhs(np.conj(f).T) for f in fs])
    d1 = np.arange(128)[None, :]
    j = np.arange(64)[:, None]
    e = lambda kk: np.exp(-2j * np.pi * ((kk * d1) % D) / D)
    df = np.zeros((4, 256, 256))
    e0, e4 = e(8 * j), e(4 + 8 * j)
    m0 = np.concatenate([e0.real, e0.imag])
    m0[64] = e(np.array([[512]]))[0].real
    df[0, :128, :128] = m0
    df[0, 128:, 128:] = np.concatenate([e4.real, e4.imag])
    for k2 in (1, 2, 3):
        a = e(k2 + 8 * j)
        b = e(8 - k2 + 8 * j)
        df[k2] = np.block([[a.real, -a.imag], [b.real, b.imag], [a.imag, a.real], [b.imag, -b.real]])
    di = np.zeros((4, 256, 256))
    i0 = 2 * m0.T.copy()
    i0[:, 0] /= 2
    i0[:, 64] /= 2
    di[0, :128, :128] = i0
    di[0, 128:, 128:] = 2 * df[0, 128:, 128:].T
    for k2 in (1, 2, 3):
        di[k2] = 2 * df[k2].T
    di /= S * D
    return [np.asarray(c, dtype=BF16) for c in (sf, si, df, di)]


def _fft(v, sign):
    n = len(v)
    if n == 1:
        return v
    ev, od = _fft(v[0::2], sign), _fft(v[1::2], sign)
    out = [None] * n
    for k in range(n // 2):
        er, ei = ev[k]
        r, i = od[k]
        if k == 0:
            out[k], out[k + n // 2] = (er + r, ei + i), (er - r, ei - i)
            continue
        if 4 * k == n:
            if sign < 0:
                out[k], out[k + n // 2] = (er + i, ei - r), (er - i, ei + r)
            else:
                out[k], out[k + n // 2] = (er - i, ei + r), (er + i, ei - r)
            continue
        c, s = float(np.cos(2 * np.pi * k / n)), float(sign * np.sin(2 * np.pi * k / n))
        if 8 * k == n or 8 * k == 3 * n:
            if c * s > 0:
                tr, ti = (r - i) * c, (r + i) * c
            else:
                tr, ti = (r + i) * c, (i - r) * c
        else:
            tr, ti = r * c - i * s, r * s + i * c
        out[k], out[k + n // 2] = (er + tr, ei + ti), (er - tr, ei - ti)
    return out


def _ln(x):
    m = jnp.mean(x, axis=0, keepdims=True)
    c = x - m
    v = jnp.mean(c * c, axis=0, keepdims=True)
    return c * lax.rsqrt(v + 1e-5)


def _loop(name, lo, hi):
    def run(f):
        with jax.named_scope(name):
            pl.loop(lo, hi)(f)
    return run


def _dot(a, b):
    return jnp.dot(a, b, preferred_element_type=F32)


def _kernel(x_hbm, wqkv_hbm, wo_hbm, wr_hbm, wi_hbm, sf_hbm, si_hbm, df_hbm, di_hbm, out_hbm,
            xb, wqkv, wo, wr, wi, sf, si, df, di, xf, xT, wT, woT, wrT, wiT, xn, oT, qkvA, qkvB,
            z1, z2, sems):
    srcs = (x_hbm, wqkv_hbm, wo_hbm, wr_hbm, wi_hbm, sf_hbm, si_hbm, df_hbm, di_hbm)
    dsts = (xb, wqkv, wo, wr, wi, sf, si, df, di)
    cps = [pltpu.make_async_copy(s_, d_, sems.at[i]) for i, (s_, d_) in enumerate(zip(srcs, dsts))]
    cps[0].start()
    cps[0].wait()
    for c in cps[1:]:
        c.start()

    @_loop('L1', 0, 16)
    def _(i):
        r = pl.ds(pl.multiple_of(i * 128, 128), 128)
        for j in range(8):
            xf[j, r, :] = xb[r, j * L:(j + 1) * L].astype(F32)

    def pro(t):
        v = jnp.concatenate([xf[j, pl.ds(t, L, stride=T), :].T for j in range(8)], axis=0)
        xT[t] = v
        xn[:, pl.ds(pl.multiple_of(t * L, L), L)] = _ln(v).astype(BF16)

    @_loop('P', 0, 4)
    def _(i):
        for j in range(4):
            pro(4 * i + j)

    cps[1].wait()
    @_loop('W', 0, 8)
    def _(g):
        for p in range(3):
            wT[g, p * 128:(p + 1) * 128, :] = wqkv[:, pl.ds(pl.multiple_of(p * D + g * 128, 128), 128)].T

    lane0 = lax.broadcasted_iota(jnp.int32, (8, L), 1) == 0

    def proj(g, dst):
        dst[...] = _dot(wT[g], xn[...])

    def attn(g, src, dst=None):
        g0 = pl.multiple_of(g * 128, 128)
        for hh in range(4):
            qr, kr, vr = hh * 32, 128 + hh * 32, 256 + hh * 32
            halo = {}
            for u in range(2, T):
                halo[u] = (pltpu.roll(src[kr:kr + 32, u * L:(u + 1) * L], 1, 1),
                           pltpu.roll(src[vr:vr + 32, u * L:(u + 1) * L], 1, 1))
            for t in range(T):
                if dst is not None and t % 8 == 0:
                    c = (hh * T + t) * 32
                    dst[:, c:c + 256] = _dot(wT[g + 1], xn[:, c:c + 256])
                q = src[qr:qr + 32, t * L:(t + 1) * L] * (DH ** -0.5)
                lg = []
                for w in range(NW):
                    u = t - 2 * w
                    k = src[kr:kr + 32, u * L:(u + 1) * L] if u >= 0 else halo[u + T][0]
                    p = q * k
                    p = (p[0:8] + p[8:16]) + (p[16:24] + p[24:32])
                    for sh in (4, 2, 1):
                        p = p + pltpu.roll(p, sh, 0)
                    if u < 0:
                        p = jnp.where(lane0, -1e9, p)
                    lg.append(p)
                m = lg[0]
                for w in range(1, NW):
                    m = jnp.maximum(m, lg[w])
                ex = [jnp.exp(a - m) for a in lg]
                inv = 1.0 / sum(ex[1:], ex[0])
                acc = None
                for w in range(NW):
                    u = t - 2 * w
                    v = src[vr:vr + 32, u * L:(u + 1) * L] if u >= 0 else halo[u + T][1]
                    c = v * jnp.concatenate([ex[w]] * 4, axis=0)
                    acc = c if acc is None else acc + c
                acc = acc * jnp.concatenate([inv] * 4, axis=0)
                oT[pl.ds(g0 + hh * 32, 32), t * L:(t + 1) * L] = acc.astype(BF16)

    def layer_a(first):
        proj(0, qkvA)

        @_loop('L2', 0, 4)
        def _(i):
            attn(2 * i, qkvA, qkvB)

            @pl.when(i < 3)
            def _():
                attn(2 * i + 1, qkvB, qkvA)

        attn(7, qkvB)

        @pl.when(first)
        def _():
            cps[2].wait()
            for g in range(8):
                woT[g * 128:(g + 1) * 128, :] = wo[:, g * 128:(g + 1) * 128].T
            for c in cps[3:]:
                c.wait()
            for src, dst in ((wr, wrT), (wi, wiT)):
                for t in range(T):
                    dst[t, 0:512, :] = src[0:512, t * L:(t + 1) * L].astype(F32)
                    dst[t, 512:640, :] = jnp.broadcast_to(src[512:513, t * L:(t + 1) * L].astype(F32), (L, L))

    def oproj(i):
        c0 = pl.multiple_of(i * 256, 256)
        y = _dot(woT[...], oT[:, pl.ds(c0, 256)])
        for j in range(2):
            xT[2 * i + j] += y[:, j * L:(j + 1) * L]

    row0 = lax.broadcasted_iota(jnp.int32, (64, L), 0) == 0
    rh = float(np.sqrt(0.5))

    def layer_b(last):
        def fwd(t):
            a = _ln(xT[t])
            x = [a[i * 128:(i + 1) * 128] for i in range(8)]
            s = [x[i] + x[i + 4] for i in range(4)]
            d = [x[i] - x[i + 4] for i in range(4)]
            e, o = s[0] + s[2], s[1] + s[3]
            p, q = (d[1] - d[3]) * rh, (d[1] + d[3]) * rh
            grp = ((e + o, e - o), (d[0] + p, -(d[2] + q)), (s[0] - s[2], s[3] - s[1]),
                   (d[0] - p, d[2] - q))
            re, im = [], []
            for k2, (u, v) in enumerate(grp):
                if k2 == 0:
                    y0 = _dot(df[0, :128, :128], u.astype(BF16))
                    y4 = _dot(df[0, 128:, 128:], v.astype(BF16))
                    re += [y0[:64], y4[:64]]
                    im += [jnp.where(row0, 0.0, y0[64:]), y4[64:]]
                    nyq = y0[64:80]
                else:
                    y = _dot(df[k2], jnp.concatenate([u, v], axis=0).astype(BF16))
                    re.append(y[:128])
                    im.append(y[128:])
            z = jnp.concatenate([jnp.concatenate(re + [nyq], axis=0),
                                 jnp.concatenate(im + [jnp.zeros_like(nyq)], axis=0)], axis=1)
            z1[t] = _dot(z.astype(BF16), sf[t])

        oproj(0)

        @_loop('L4', 0, 7)
        def _(i):
            oproj(i + 1)
            fwd(2 * i)
            fwd(2 * i + 1)

        fwd(14)
        fwd(15)

        def mid(r0, w0):
            res = []
            for hf in range(2):
                rows = pl.ds(r0 + 8 * hf, 8)
                f = _fft([(z1[t, rows, :L], z1[t, rows, L:]) for t in range(T)], -1)
                wrows = pl.ds(w0 + 64 * hf, 8, stride=8)
                g = []
                for k in range(T):
                    a, b = wrT[k, wrows, :], wiT[k, wrows, :]
                    g.append((f[k][0] * a - f[k][1] * b, f[k][0] * b + f[k][1] * a))
                res.append(_fft(g, 1))
            for t in range(T):
                for c in range(2):
                    z2[t, pl.ds(r0, 16), c * L:(c + 1) * L] = jnp.concatenate(
                        [res[0][t][c], res[1][t][c]], axis=0).astype(BF16)

        for b, r in enumerate(RES):
            @_loop('L5', 0, 5 if b == 0 else 4)
            def _(i):
                r0 = jnp.where(i == 4, 512, b * 64 + i * 16) if b == 0 else b * 64 + i * 16
                mid(pl.multiple_of(r0, 16), r + pl.multiple_of(i * 128, 128))

        def inv(t):
            u = _dot(z2[t], si[t])
            ur, ui = u[:, :L], u[:, L:]
            nyq = jnp.concatenate([ur[512:528]] * 4, axis=0)
            c0 = _dot(di[0, :128, :128], jnp.concatenate(
                [ur[:64], jnp.where(row0, nyq, ui[:64])], axis=0).astype(BF16))
            c4 = _dot(di[0, 128:, 128:], jnp.concatenate(
                [ur[64:128], ui[64:128]], axis=0).astype(BF16))
            c = []
            for k2 in (1, 2, 3):
                r = slice(k2 * 128, (k2 + 1) * 128)
                y = _dot(di[k2], jnp.concatenate([ur[r], ui[r]], axis=0).astype(BF16))
                c.append((y[:128], y[128:]))
            (r1, i1), (r2, i2), (r3, i3) = c
            e, o = c0 + c4, c0 - c4
            s = [e + r2, o - i2, e - r2, o + i2]
            p, q = (r1 - r3) * rh, (i1 + i3) * rh
            d = [r1 + r3, p - q, i3 - i1, -(p + q)]
            y = jnp.concatenate([s[i] + d[i] for i in range(4)] + [s[i] - d[i] for i in range(4)], axis=0)
            v = xT[t] + y
            xT[t] = v
            xn[:, pl.ds(pl.multiple_of(t * L, L), L)] = _ln(v).astype(BF16)

        @_loop('L6', 0, 4)
        def _(i):
            for j in range(4):
                inv(4 * i + j)

    @_loop('L7', 0, 2)
    def _(it):
        with jax.named_scope('A'):
            layer_a(it == 0)
        with jax.named_scope('B'):
            layer_b(it == 1)

    @_loop('E', 0, T)
    def _(t):
        for j in range(8):
            xf[j, pl.ds(t, L, stride=T), :] = xT[t, j * L:(j + 1) * L, :].T
    oc = [pltpu.make_async_copy(xb.at[i * 256:(i + 1) * 256], out_hbm.at[i * 256:(i + 1) * 256], sems.at[i])
          for i in range(8)]
    for i in range(8):
        for j in range(8):
            xb[i * 256:(i + 1) * 256, j * L:(j + 1) * L] = xf[j, i * 256:(i + 1) * 256, :].astype(BF16)
        oc[i].start()
    for c in oc:
        c.wait()


@jax.jit
def pallas_interleave_layers__sliding_local_dilated__spectral_gfnet__prompt_kernel(
    A_x, A_wqkv, A_wo, B_x, B_w_r, B_w_i,
):
    del B_x
    V = pltpu.VMEM
    out = pl.pallas_call(
        _kernel,
        out_shape=jax.ShapeDtypeStruct((S, D), BF16),
        in_specs=[pl.BlockSpec(memory_space=pl.ANY)] * 9,
        out_specs=pl.BlockSpec(memory_space=pl.ANY),
        scratch_shapes=[
            V((S, D), BF16), V((D, 3 * D), BF16), V((D, D), BF16), V((513, S), BF16), V((513, S), BF16),
            V((T, 256, 256), BF16), V((T, 256, 256), BF16), V((4, 256, 256), BF16), V((4, 256, 256), BF16),
            V((8, S, L), F32), V((T, D, L), F32), V((8, 384, D), BF16), V((D, D), BF16),
            V((T, 640, L), F32), V((T, 640, L), F32), V((D, S), BF16), V((D, S), BF16),
            V((384, S), F32), V((384, S), F32), V((T, ZR, 256), F32), V((T, ZR, 256), BF16),
            pltpu.SemaphoreType.DMA((9,)),
        ],
        compiler_params=pltpu.CompilerParams(vmem_limit_bytes=120 * 1024 * 1024),
    )(A_x.reshape(S, D), A_wqkv, A_wo, B_w_r.T, B_w_i.T, *_consts())
    return out.reshape(1, S, D)
```
